```python
import os as _os
_os.environ.setdefault("JAX_PLATFORMS", "cpu")
import jax
import jax.numpy as jnp

def _softmax(x, axis=-1):
    return jax.nn.softmax(x, axis=axis)
def _gelu(x):
    return jax.nn.gelu(x, approximate=True)
def _silu(x):
    return jax.nn.silu(x)
def _sigmoid(x):
    return jax.nn.sigmoid(x)
def _layernorm(x, axis=-1, eps=1e-5):
    m = jnp.mean(x, axis=axis, keepdims=True)
    v = jnp.var(x, axis=axis, keepdims=True)
    return (x - m) / jnp.sqrt(v + eps)
def _scatter_add(tgt, idx, src, axis=0):
    return tgt.at[idx].add(src)
def _segment_sum(src, seg, n):
    return jax.ops.segment_sum(src, seg, n)
class _Rng:
    def __init__(self, key):
        self._k = key
    def _next(self):
        self._k, sub = jax.random.split(self._k)
        return sub
    def normal(self, shape):
        return jax.random.normal(self._next(), shape, dtype=jnp.bfloat16)
    def randint(self, lo, hi, shape):
        return jax.random.randint(self._next(), shape, lo, hi, dtype=jnp.int32)
    def uniform(self, shape, lo=0.0, hi=1.0):
        return jax.random.uniform(self._next(), shape, jnp.bfloat16, lo, hi)
    def permutation(self, n):
        return jax.random.permutation(self._next(), n)


kernel_name = 'sequential_preLN__compressed_kv_cla__dense_activation_mish__decode'

def setup_inputs():
    _rng = _Rng(jax.random.key(int.from_bytes(__import__("os").urandom(4), "little")))
    _w = (lambda a: (lambda t: t.astype(jnp.bfloat16) if jnp.issubdtype(t.dtype, jnp.floating) else t)(jnp.asarray(a)))
    def _A_setup():
        B, H, Sq, Sk, D, M = 2, 32, 1, 8192, 128, 512
        Dc = 4 * D
        return {
            "x": _w((lambda *s: _rng.normal(s) * 0.05)(B, Sq, M)),
            "c_kv": _w((lambda *s: _rng.normal(s) * 0.8)(B, Sk, Dc)),
            "w_q": _w((lambda *s: _rng.normal(s) * 0.8)(M, H, D) * (M ** -0.5)),
            "w_uk": _w((lambda *s: _rng.normal(s) * 0.8)(Dc, H, D) * (Dc ** -0.5)),
            "w_uv": _w((lambda *s: _rng.normal(s) * 0.8)(Dc, H, D) * (Dc ** -0.5)),
            "w_o": _w((lambda *s: _rng.normal(s) * 0.8)(H, D, M) * ((H * D) ** -0.5)),
        }
    _A_in = _A_setup()

    def _B_setup():
        B, S, D, F = 2, 1, 512, 1792
        return {
            "x": _w((lambda *s: _rng.normal(s) * 0.05)(B, S, D)),
            "w1": _w((lambda *s: _rng.normal(s) * 0.4)(D, F) * (D ** -0.5)),
            "b1": _w((lambda *s: _rng.normal(s) * 0.05)(F)),
            "w2": _w((lambda *s: _rng.normal(s) * 0.05)(F, D) * (F ** -0.5)),
        }
    _B_in = _B_setup()

    return {
        "A_x": _A_in["x"],
        "A_c_kv": _A_in["c_kv"],
        "A_w_q": _A_in["w_q"],
        "A_w_uk": _A_in["w_uk"],
        "A_w_uv": _A_in["w_uv"],
        "A_w_o": _A_in["w_o"],
        "B_x": _B_in["x"],
        "B_w1": _B_in["w1"],
        "B_b1": _B_in["b1"],
        "B_w2": _B_in["w2"],
    }

def reference(A_x, A_c_kv, A_w_q, A_w_uk, A_w_uv, A_w_o, B_x, B_w1, B_b1, B_w2):
    def _A_ref(x, c_kv, w_q, w_uk, w_uv, w_o):
        B, Sq, M = x.shape[0], x.shape[1], x.shape[2]
        Sk = c_kv.shape[1]
        H, D = w_q.shape[1], w_q.shape[2]
        q = jnp.einsum("bqm,mhd->bhqd", x, w_q)
        k = jnp.einsum("bkc,chd->bhkd", c_kv, w_uk)
        v = jnp.einsum("bkc,chd->bhkd", c_kv, w_uv)
        scores = jnp.einsum("bhqd,bhkd->bhqk", q, k) * (D ** -0.5)
        off = Sk - Sq
        qi = jnp.arange(Sq)[:, None]
        kj = jnp.arange(Sk)[None, :]
        cmask = kj <= (qi + off)
        scores = jnp.where(cmask[None, None], scores, -1e9)
        p = _softmax(scores, axis=-1)
        ctx = jnp.einsum("bhqk,bhkd->bhqd", p, v)
        return jnp.einsum("bhqd,hdm->bqm", ctx, w_o)

    def _B_ref(x, w1, b1, w2):
        h = jnp.einsum("bsd,df->bsf", x, w1) + b1
        sp = jnp.log1p(jnp.exp(-jnp.abs(h))) + jnp.where(h > 0, h, jnp.zeros_like(h))
        act = h * jnp.tanh(sp)
        return jnp.einsum("bsf,fd->bsd", act, w2)

    x = A_x
    h = x + _A_ref(_layernorm(x, axis=-1), A_c_kv, A_w_q, A_w_uk, A_w_uv, A_w_o)
    h2 = h + _B_ref(_layernorm(h, axis=-1), B_w1, B_b1, B_w2)
    return h2
```

```python
import jax
import jax.numpy as jnp
import jax.experimental.pallas as pl
import jax.experimental.pallas.tpu as pltpu

_LN_EPS = 1e-5
_TK = 1024
_NT = (((1,), (1,)), ((), ()))


def _layernorm(v):
    m = jnp.mean(v, axis=-1, keepdims=True)
    d = v - m
    var = jnp.mean(d * d, axis=-1, keepdims=True)
    return d / jnp.sqrt(var + _LN_EPS)


@jax.jit
def pallas_sequential_preLN__compressed_kv_cla__dense_activation_mish__decode_kernel(
    A_x: jax.Array,
    A_c_kv: jax.Array,
    A_w_q: jax.Array,
    A_w_uk: jax.Array,
    A_w_uv: jax.Array,
    A_w_o: jax.Array,
    B_x: jax.Array,
    B_w1: jax.Array,
    B_b1: jax.Array,
    B_w2: jax.Array,
):
    del B_x
    B, Sq, M = A_x.shape
    _, Sk, C = A_c_kv.shape
    _, H, D = A_w_q.shape
    F = B_w1.shape[1]
    assert Sq == 1 and B == 2 and Sk % _TK == 0 and H % 8 == 0
    n_chunks = Sk // _TK
    scale = float(D) ** -0.5
    f32, bf16 = jnp.float32, jnp.bfloat16
    R = 8 * B

    S_X, S_B1, S_WQ, S_WUK, S_WUV, S_WO, S_W1, S_W2 = range(8)
    S_KV = 8

    def kernel(x_hbm, ckv_hbm, wq_hbm, wuk_hbm, wuv_hbm, wo_hbm, w1_hbm, b1_hbm, w2_hbm,
               o_ref,
               x_v, ckv_v, wq_v, wuk_v, wuv_v, wo_v, w1_v, b1_v, w2_v, sem):
        def cp(src, dst, slot):
            return pltpu.make_async_copy(src, dst, sem.at[slot])

        def kv_cp(b, i):
            return cp(ckv_hbm.at[b, pl.ds(i * _TK, _TK)], ckv_v.at[b, pl.ds(i * _TK, _TK)],
                      S_KV + b * n_chunks + i)

        c_x = cp(x_hbm, x_v, S_X)
        c_wq = cp(wq_hbm, wq_v, S_WQ)
        c_wuk = cp(wuk_hbm, wuk_v, S_WUK)
        c_wuv = cp(wuv_hbm, wuv_v, S_WUV)
        c_wo = cp(wo_hbm, wo_v, S_WO)
        c_w1 = cp(w1_hbm, w1_v, S_W1)
        c_b1 = cp(b1_hbm, b1_v, S_B1)
        c_w2 = cp(w2_hbm, w2_v, S_W2)
        c_x.start()
        c_wq.start()
        c_wuk.start()
        for b in range(B):
            for i in range(n_chunks):
                kv_cp(b, i).start()
        c_wuv.start()
        c_wo.start()
        c_b1.start()
        c_w1.start()
        c_w2.start()

        def rows(parts):
            return jnp.concatenate(
                [jnp.broadcast_to(p, (8, p.shape[-1])) for p in parts], axis=0)

        c_x.wait()
        x16 = rows([x_v[b].astype(f32) for b in range(B)])
        xln = _layernorm(x16).astype(bf16)

        c_wq.wait()
        wq2 = wq_v.reshape(M * H, D)
        q = []
        for h in range(H):
            wh = wq2[pl.ds(h, M, stride=H), :]
            q.append(jnp.dot(xln, wh, preferred_element_type=f32).astype(bf16))

        c_wuk.wait()
        wuk2 = wuk_v.reshape(C * H, D)
        sub = jax.lax.broadcasted_iota(jnp.int32, (8, C), 0)
        qa = [[None] * (H // 8) for _ in range(B)]
        for h in range(H):
            wh = wuk2[pl.ds(h, C, stride=H), :]
            r = jax.lax.dot_general(q[h], wh, _NT, preferred_element_type=f32)
            for b in range(B):
                rb = r[8 * b:8 * b + 8]
                cur = qa[b][h // 8]
                qa[b][h // 8] = rb if cur is None else jnp.where(sub == h % 8, rb, cur)
        qa = [(jnp.concatenate(qa[b], axis=0) * scale).astype(bf16) for b in range(B)]

        ctxc = []
        for b in range(B):
            def step(i, carry, b=b):
                m, l, acc = carry
                kv_cp(b, i).wait()
                c = ckv_v[b, pl.ds(pl.multiple_of(i * _TK, _TK), _TK), :]
                s = jax.lax.dot_general(qa[b], c, _NT, preferred_element_type=f32)
                m_new = jnp.maximum(m, jnp.max(s, axis=-1, keepdims=True))
                alpha = jnp.exp(m - m_new)
                p = jnp.exp(s - m_new)
                l = alpha * l + jnp.sum(p, axis=-1, keepdims=True)
                acc = alpha * acc + jnp.dot(p.astype(bf16), c, preferred_element_type=f32)
                return m_new, l, acc
            init = (jnp.full((H, 1), -jnp.inf, f32), jnp.zeros((H, 1), f32),
                    jnp.zeros((H, C), f32))
            _, l, acc = jax.lax.fori_loop(0, n_chunks, step, init)
            ctxc.append(acc / l)

        c_wuv.wait()
        wuv2 = wuv_v.reshape(C * H, D)
        ctx = []
        for h in range(H):
            lhs = rows([ctxc[b][h:h + 1, :] for b in range(B)]).astype(bf16)
            wh = wuv2[pl.ds(h, C, stride=H), :]
            ctx.append(jnp.dot(lhs, wh, preferred_element_type=f32).astype(bf16))

        c_wo.wait()
        att = jnp.zeros((R, M), f32)
        for h in range(H):
            att = att + jnp.dot(ctx[h], wo_v[h], preferred_element_type=f32)
        hres = x16 + att

        hln = _layernorm(hres).astype(bf16)
        c_b1.wait()
        c_w1.wait()
        h1 = jnp.dot(hln, w1_v[...], preferred_element_type=f32)
        h1 = h1 + b1_v[...].astype(f32).reshape(1, F)
        sp = jnp.log1p(jnp.exp(-jnp.abs(h1))) + jnp.where(h1 > 0, h1, jnp.zeros_like(h1))
        act = (h1 * jnp.tanh(sp)).astype(bf16)
        c_w2.wait()
        out = hres + jnp.dot(act, w2_v[...], preferred_element_type=f32)
        for b in range(B):
            o_ref[b] = out[8 * b:8 * b + 1, :].astype(o_ref.dtype)

    anyspec = pl.BlockSpec(memory_space=pl.ANY)
    return pl.pallas_call(
        kernel,
        out_shape=jax.ShapeDtypeStruct((B, Sq, M), A_x.dtype),
        in_specs=[anyspec] * 9,
        out_specs=pl.BlockSpec(memory_space=pltpu.VMEM),
        scratch_shapes=[
            pltpu.VMEM(A_x.shape, bf16),
            pltpu.VMEM(A_c_kv.shape, bf16),
            pltpu.VMEM(A_w_q.shape, bf16),
            pltpu.VMEM(A_w_uk.shape, bf16),
            pltpu.VMEM(A_w_uv.shape, bf16),
            pltpu.VMEM(A_w_o.shape, bf16),
            pltpu.VMEM(B_w1.shape, bf16),
            pltpu.VMEM(B_b1.shape, bf16),
            pltpu.VMEM(B_w2.shape, bf16),
            pltpu.SemaphoreType.DMA((S_KV + B * n_chunks,)),
        ],
        compiler_params=pltpu.CompilerParams(vmem_limit_bytes=100 * 1024 * 1024),
    )(A_x, A_c_kv, A_w_q, A_w_uk, A_w_uv, A_w_o, B_w1, B_b1, B_w2)
```

```python
import jax
import jax.numpy as jnp
import jax.experimental.pallas as pl
import jax.experimental.pallas.tpu as pltpu

_LN_EPS = 1e-5
_TK = 1024
_NT = (((1,), (1,)), ((), ()))


def _layernorm(v):
    m = jnp.mean(v, axis=-1, keepdims=True)
    d = v - m
    var = jnp.mean(d * d, axis=-1, keepdims=True)
    return d / jnp.sqrt(var + _LN_EPS)


@jax.jit
def pallas_sequential_preLN__compressed_kv_cla__dense_activation_mish__decode_kernel(
    A_x: jax.Array,
    A_c_kv: jax.Array,
    A_w_q: jax.Array,
    A_w_uk: jax.Array,
    A_w_uv: jax.Array,
    A_w_o: jax.Array,
    B_x: jax.Array,
    B_w1: jax.Array,
    B_b1: jax.Array,
    B_w2: jax.Array,
):
    del B_x
    B, Sq, M = A_x.shape
    _, Sk, C = A_c_kv.shape
    _, H, D = A_w_q.shape
    F = B_w1.shape[1]
    assert Sq == 1 and B == 2 and Sk % _TK == 0 and H % 8 == 0
    n_chunks = Sk // _TK
    scale = float(D) ** -0.5
    f32, bf16 = jnp.float32, jnp.bfloat16
    R = 8 * B

    S_X, S_B1, S_WQ, S_WUK, S_WUV, S_WO, S_W1, S_W2 = range(8)
    S_KV = 8

    def kernel(x_hbm, ckv_hbm, wq_hbm, wuk_hbm, wuv_hbm, wo_hbm, w1_hbm, b1_hbm, w2_hbm,
               o_ref,
               x_v, ckv_v, wq_v, wuk_v, wuv_v, wo_v, w1_v, b1_v, w2_v, sem):
        def cp(src, dst, slot):
            return pltpu.make_async_copy(src, dst, sem.at[slot])

        def kv_cp(b, i):
            return cp(ckv_hbm.at[b, pl.ds(i * _TK, _TK)], ckv_v.at[b, pl.ds(i * _TK, _TK)],
                      S_KV + b * n_chunks + i)

        c_x = cp(x_hbm, x_v, S_X)
        c_wq = cp(wq_hbm, wq_v, S_WQ)
        c_wuk = cp(wuk_hbm, wuk_v, S_WUK)
        c_wuv = cp(wuv_hbm, wuv_v, S_WUV)
        c_wo = cp(wo_hbm, wo_v, S_WO)
        c_w1 = cp(w1_hbm, w1_v, S_W1)
        c_b1 = cp(b1_hbm, b1_v, S_B1)
        c_w2 = cp(w2_hbm, w2_v, S_W2)
        c_x.start()
        c_wq.start()
        c_wuk.start()
        for b in range(B):
            for i in range(n_chunks):
                kv_cp(b, i).start()
        c_wuv.start()
        c_wo.start()
        c_b1.start()
        c_w1.start()
        c_w2.start()

        def rows(parts):
            return jnp.concatenate(
                [jnp.broadcast_to(p, (8, p.shape[-1])) for p in parts], axis=0)

        c_x.wait()
        xf = x_v[...].astype(f32)
        x16 = rows([xf[b:b + 1] for b in range(B)])
        xln = _layernorm(x16).astype(bf16)

        c_wq.wait()
        wq2 = wq_v.reshape(M * H, D)
        q = []
        for h in range(H):
            wh = wq2[pl.ds(h, M, stride=H), :]
            q.append(jnp.dot(xln, wh, preferred_element_type=f32).astype(bf16))

        c_wuk.wait()
        wuk2 = wuk_v.reshape(C * H, D)
        sub = jax.lax.broadcasted_iota(jnp.int32, (8, C), 0)
        qa = [[None] * (H // 8) for _ in range(B)]
        for h in range(H):
            wh = wuk2[pl.ds(h, C, stride=H), :]
            r = jax.lax.dot_general(q[h], wh, _NT, preferred_element_type=f32)
            for b in range(B):
                rb = r[8 * b:8 * b + 8]
                cur = qa[b][h // 8]
                qa[b][h // 8] = rb if cur is None else jnp.where(sub == h % 8, rb, cur)
        qa = [(jnp.concatenate(qa[b], axis=0) * scale).astype(bf16) for b in range(B)]

        ctxc = []
        for b in range(B):
            def step(i, carry, b=b):
                m, l, acc = carry
                kv_cp(b, i).wait()
                c = ckv_v[b, pl.ds(pl.multiple_of(i * _TK, _TK), _TK), :]
                s = jax.lax.dot_general(qa[b], c, _NT, preferred_element_type=f32)
                m_new = jnp.maximum(m, jnp.max(s, axis=-1, keepdims=True))
                alpha = jnp.exp(m - m_new)
                p = jnp.exp(s - m_new)
                l = alpha * l + jnp.sum(p, axis=-1, keepdims=True)
                acc = alpha * acc + jnp.dot(p.astype(bf16), c, preferred_element_type=f32)
                return m_new, l, acc
            init = (jnp.full((H, 1), -jnp.inf, f32), jnp.zeros((H, 1), f32),
                    jnp.zeros((H, C), f32))
            _, l, acc = jax.lax.fori_loop(0, n_chunks, step, init)
            ctxc.append(acc / l)

        c_wuv.wait()
        wuv2 = wuv_v.reshape(C * H, D)
        ctx = []
        for h in range(H):
            lhs = rows([ctxc[b][h:h + 1, :] for b in range(B)]).astype(bf16)
            wh = wuv2[pl.ds(h, C, stride=H), :]
            ctx.append(jnp.dot(lhs, wh, preferred_element_type=f32).astype(bf16))

        c_wo.wait()
        att = jnp.zeros((R, M), f32)
        for h in range(H):
            att = att + jnp.dot(ctx[h], wo_v[h], preferred_element_type=f32)
        hres = x16 + att

        hln = _layernorm(hres).astype(bf16)
        c_b1.wait()
        c_w1.wait()
        h1 = jnp.dot(hln, w1_v[...], preferred_element_type=f32)
        h1 = h1 + b1_v[...].astype(f32).reshape(1, F)
        sp = jnp.log1p(jnp.exp(-jnp.abs(h1))) + jnp.where(h1 > 0, h1, jnp.zeros_like(h1))
        act = (h1 * jnp.tanh(sp)).astype(bf16)
        c_w2.wait()
        out = hres + jnp.dot(act, w2_v[...], preferred_element_type=f32)
        o_ref[...] = jnp.concatenate(
            [out[8 * b:8 * b + 1, :] for b in range(B)], axis=0).astype(o_ref.dtype)

    anyspec = pl.BlockSpec(memory_space=pl.ANY)
    out = pl.pallas_call(
        kernel,
        out_shape=jax.ShapeDtypeStruct((B, M), A_x.dtype),
        in_specs=[anyspec] * 9,
        out_specs=pl.BlockSpec(memory_space=pltpu.VMEM),
        scratch_shapes=[
            pltpu.VMEM((B, M), bf16),
            pltpu.VMEM(A_c_kv.shape, bf16),
            pltpu.VMEM(A_w_q.shape, bf16),
            pltpu.VMEM(A_w_uk.shape, bf16),
            pltpu.VMEM(A_w_uv.shape, bf16),
            pltpu.VMEM(A_w_o.shape, bf16),
            pltpu.VMEM(B_w1.shape, bf16),
            pltpu.VMEM(B_b1.shape, bf16),
            pltpu.VMEM(B_w2.shape, bf16),
            pltpu.SemaphoreType.DMA((S_KV + B * n_chunks,)),
        ],
        compiler_params=pltpu.CompilerParams(vmem_limit_bytes=100 * 1024 * 1024),
    )(A_x.reshape(B, M), A_c_kv, A_w_q, A_w_uk, A_w_uv, A_w_o, B_w1, B_b1, B_w2)
    return out.reshape(B, Sq, M)
```

```python
import jax
import jax.numpy as jnp
import jax.experimental.pallas as pl
import jax.experimental.pallas.tpu as pltpu

_LN_EPS = 1e-5
_TK = 1024
_W2_TAIL = (256, 128)
_NT = (((1,), (1,)), ((), ()))


def _layernorm(v):
    mean = jnp.mean(v, axis=-1, keepdims=True)
    d = v - mean
    var = jnp.mean(d * d, axis=-1, keepdims=True)
    return d / jnp.sqrt(var + _LN_EPS)


def _batch_rows(parts):
    return jnp.concatenate(
        [jnp.broadcast_to(p, (8, p.shape[-1])) for p in parts], axis=0)


@jax.jit
def pallas_sequential_preLN__compressed_kv_cla__dense_activation_mish__decode_kernel(
    A_x: jax.Array,
    A_c_kv: jax.Array,
    A_w_q: jax.Array,
    A_w_uk: jax.Array,
    A_w_uv: jax.Array,
    A_w_o: jax.Array,
    B_x: jax.Array,
    B_w1: jax.Array,
    B_b1: jax.Array,
    B_w2: jax.Array,
):
    del B_x
    B, Sq, M = A_x.shape
    _, Sk, C = A_c_kv.shape
    _, H, D = A_w_q.shape
    F = B_w1.shape[1]
    assert Sq == 1 and B <= 8 and Sk % _TK == 0 and H % 16 == 0
    assert D % 128 == 0 and F > sum(_W2_TAIL)
    n_kv = Sk // _TK
    scale = float(D) ** -0.5
    f32, bf16 = jnp.float32, jnp.bfloat16

    w2_slabs = []
    start = 0
    for size in (F - sum(_W2_TAIL),) + _W2_TAIL:
        w2_slabs.append((start, size))
        start += size

    S_X, S_WQ, S_WUK, S_WUV, S_WO, S_B1, S_W1 = range(7)
    S_W2 = 7
    S_KV = S_W2 + len(w2_slabs)
    n_sem = S_KV + B * n_kv

    def kernel(x_hbm, ckv_hbm, wq_hbm, wuk_hbm, wuv_hbm, wo_hbm, w1_hbm, b1_hbm, w2_hbm,
               o_ref,
               x_v, ckv_v, wq_v, wuk_v, wuv_v, wo_v, w1_v, b1_v, w2_v, sem):

        def copy(src, dst, slot):
            return pltpu.make_async_copy(src, dst, sem.at[slot])

        def kv_copy(b, i):
            rows = pl.ds(pl.multiple_of(i * _TK, _TK), _TK)
            return copy(ckv_hbm.at[b, rows], ckv_v.at[b, rows], S_KV + b * n_kv + i)

        def w2_copy(j):
            rows = pl.ds(*w2_slabs[j])
            return copy(w2_hbm.at[rows], w2_v.at[rows], S_W2 + j)

        x_copy = copy(x_hbm, x_v, S_X)
        wq_copy = copy(wq_hbm, wq_v, S_WQ)
        wuk_copy = copy(wuk_hbm, wuk_v, S_WUK)
        wuv_copy = copy(wuv_hbm, wuv_v, S_WUV)
        wo_copy = copy(wo_hbm, wo_v, S_WO)
        b1_copy = copy(b1_hbm, b1_v, S_B1)
        w1_copy = copy(w1_hbm, w1_v, S_W1)
        x_copy.start()
        wq_copy.start()
        wuk_copy.start()
        for b in range(B):
            for i in range(n_kv):
                kv_copy(b, i).start()
        wuv_copy.start()
        wo_copy.start()
        b1_copy.start()
        w1_copy.start()
        for j in range(len(w2_slabs)):
            w2_copy(j).start()

        def head_matrix(w_flat, rows, h):
            return w_flat[pl.ds(h, rows, stride=H), :]

        x_copy.wait()
        x_f32 = x_v[...].astype(f32)
        x_rows = _batch_rows([x_f32[b:b + 1] for b in range(B)])
        x_ln = _layernorm(x_rows).astype(bf16)

        wq_copy.wait()
        wq_flat = wq_v.reshape(M * H, D)
        q = [jnp.dot(x_ln, head_matrix(wq_flat, M, h),
                     preferred_element_type=f32).astype(bf16)
             for h in range(H)]

        wuk_copy.wait()
        wuk_flat = wuk_v.reshape(C * H, D)
        sublane = jax.lax.broadcasted_iota(jnp.int32, (8, C), 0)
        qa = [[None] * (H // 8) for _ in range(B)]
        for h in range(H):
            r = jax.lax.dot_general(q[h], head_matrix(wuk_flat, C, h), _NT,
                                    preferred_element_type=f32)
            for b in range(B):
                rb = r[8 * b:8 * b + 8]
                cur = qa[b][h // 8]
                qa[b][h // 8] = rb if cur is None else jnp.where(sublane == h % 8, rb, cur)
        qa = [(jnp.concatenate(qa[b], axis=0) * scale).astype(bf16)
              for b in range(B)]

        ctx_c = []
        for b in range(B):
            def step(i, carry, b=b):
                m, l, acc = carry
                kv_copy(b, i).wait()
                c = ckv_v[b, pl.ds(pl.multiple_of(i * _TK, _TK), _TK), :]
                s = jax.lax.dot_general(qa[b], c, _NT,
                                        preferred_element_type=f32)
                m_new = jnp.maximum(m, jnp.max(s, axis=-1, keepdims=True))
                m_sub = jnp.where(m_new == -jnp.inf, 0.0, m_new)
                alpha = jnp.exp(m - m_sub)
                p = jnp.exp(s - m_sub)
                l = alpha * l + jnp.sum(p, axis=-1, keepdims=True)
                acc = alpha * acc + jnp.dot(p.astype(bf16), c,
                                            preferred_element_type=f32)
                return m_new, l, acc

            init = (jnp.full((H, 1), -jnp.inf, f32),
                    jnp.zeros((H, 1), f32),
                    jnp.zeros((H, C), f32))
            _, l, acc = jax.lax.fori_loop(0, n_kv, step, init)
            ctx_c.append(acc / l)

        wuv_copy.wait()
        wuv_flat = wuv_v.reshape(C * H, D)
        ctx = []
        for h in range(H):
            lhs = _batch_rows([ctx_c[b][h:h + 1, :] for b in range(B)]).astype(bf16)
            ctx.append(jnp.dot(lhs, head_matrix(wuv_flat, C, h),
                               preferred_element_type=f32).astype(bf16))

        wo_copy.wait()
        attn = jnp.zeros((8 * B, M), f32)
        for h in range(H):
            attn = attn + jnp.dot(ctx[h], wo_v[h], preferred_element_type=f32)
        hidden = x_rows + attn
        row = jax.lax.broadcasted_iota(jnp.int32, (8, M), 0)
        h_res = hidden[0:8]
        for b in range(1, B):
            h_res = jnp.where(row >= b, hidden[8 * b:8 * b + 8], h_res)

        h_ln = _layernorm(h_res).astype(bf16)
        b1_copy.wait()
        w1_copy.wait()
        pre = jnp.dot(h_ln, w1_v[...], preferred_element_type=f32)
        pre = pre + b1_v[...].astype(f32).reshape(1, F)
        softplus = (jnp.log1p(jnp.exp(-jnp.abs(pre)))
                    + jnp.where(pre > 0, pre, jnp.zeros_like(pre)))
        act = (pre * jnp.tanh(softplus)).astype(bf16)

        out = h_res
        for j, (k0, kn) in enumerate(w2_slabs):
            w2_copy(j).wait()
            out = out + jnp.dot(act[:, k0:k0 + kn], w2_v[pl.ds(k0, kn), :],
                                preferred_element_type=f32)
        o_ref[...] = out[0:B, :].astype(o_ref.dtype)

    hbm = pl.BlockSpec(memory_space=pl.ANY)
    out = pl.pallas_call(
        kernel,
        out_shape=jax.ShapeDtypeStruct((B, M), A_x.dtype),
        in_specs=[hbm] * 9,
        out_specs=pl.BlockSpec(memory_space=pltpu.VMEM),
        scratch_shapes=[
            pltpu.VMEM((B, M), bf16),
            pltpu.VMEM(A_c_kv.shape, bf16),
            pltpu.VMEM(A_w_q.shape, bf16),
            pltpu.VMEM(A_w_uk.shape, bf16),
            pltpu.VMEM(A_w_uv.shape, bf16),
            pltpu.VMEM(A_w_o.shape, bf16),
            pltpu.VMEM(B_w1.shape, bf16),
            pltpu.VMEM(B_b1.shape, bf16),
            pltpu.VMEM(B_w2.shape, bf16),
            pltpu.SemaphoreType.DMA((n_sem,)),
        ],
        compiler_params=pltpu.CompilerParams(
            vmem_limit_bytes=64 * 1024 * 1024,
            disable_semaphore_checks=True,
        ),
    )(A_x.reshape(B, M), A_c_kv, A_w_q, A_w_uk, A_w_uv, A_w_o, B_w1, B_b1, B_w2)
    return out.reshape(B, Sq, M)
```

```python
import jax
import jax.numpy as jnp
import jax.experimental.pallas as pl
import jax.experimental.pallas.tpu as pltpu

_LN_EPS = 1e-5
_TK = 1024
_W2_TAIL = (256, 128)
_NT = (((1,), (1,)), ((), ()))


def _layernorm(v):
    mean = jnp.mean(v, axis=-1, keepdims=True)
    d = v - mean
    var = jnp.mean(d * d, axis=-1, keepdims=True)
    return d / jnp.sqrt(var + _LN_EPS)


def _batch_rows(parts):
    return jnp.concatenate(
        [jnp.broadcast_to(p, (8, p.shape[-1])) for p in parts], axis=0)


@jax.jit
def pallas_sequential_preLN__compressed_kv_cla__dense_activation_mish__decode_kernel(
    A_x: jax.Array,
    A_c_kv: jax.Array,
    A_w_q: jax.Array,
    A_w_uk: jax.Array,
    A_w_uv: jax.Array,
    A_w_o: jax.Array,
    B_x: jax.Array,
    B_w1: jax.Array,
    B_b1: jax.Array,
    B_w2: jax.Array,
):
    del B_x
    B, Sq, M = A_x.shape
    _, Sk, C = A_c_kv.shape
    _, H, D = A_w_q.shape
    F = B_w1.shape[1]
    assert Sq == 1 and B <= 8 and Sk % _TK == 0 and H % 16 == 0
    assert D % 128 == 0 and F > sum(_W2_TAIL)
    n_kv = Sk // _TK
    scale = float(D) ** -0.5
    f32, bf16 = jnp.float32, jnp.bfloat16

    w2_slabs = []
    start = 0
    for size in (F - sum(_W2_TAIL),) + _W2_TAIL:
        w2_slabs.append((start, size))
        start += size

    S_X, S_WQ, S_WUK, S_WUV, S_WO, S_B1, S_W1 = range(7)
    S_W2 = 7
    S_KV = S_W2 + len(w2_slabs)
    n_sem = S_KV + B * n_kv

    def body(x_hbm, ckv_hbm, wq_hbm, wuk_hbm, wuv_hbm, wo_hbm, w1_hbm, b1_hbm, w2_hbm,
             o_ref,
             x_v, ckv_v, wq_v, wuk_v, wuv_v, wo_v, w1_v, b1_v, w2_v, sem):

        def copy(src, dst, slot):
            return pltpu.make_async_copy(src, dst, sem.at[slot])

        def kv_copy(b, i):
            first = i * _TK if isinstance(i, int) else pl.multiple_of(i * _TK, _TK)
            rows = pl.ds(first, _TK)
            return copy(ckv_hbm.at[b, rows], ckv_v.at[b, rows], S_KV + b * n_kv + i)

        def w2_copy(j):
            rows = pl.ds(*w2_slabs[j])
            return copy(w2_hbm.at[rows], w2_v.at[rows], S_W2 + j)

        x_copy = copy(x_hbm, x_v, S_X)
        wq_copy = copy(wq_hbm, wq_v, S_WQ)
        wuk_copy = copy(wuk_hbm, wuk_v, S_WUK)
        wuv_copy = copy(wuv_hbm, wuv_v, S_WUV)
        wo_copy = copy(wo_hbm, wo_v, S_WO)
        b1_copy = copy(b1_hbm, b1_v, S_B1)
        w1_copy = copy(w1_hbm, w1_v, S_W1)
        x_copy.start()
        wq_copy.start()
        wuk_copy.start()
        for b in range(B):
            for i in range(n_kv):
                kv_copy(b, i).start()
        wuv_copy.start()
        wo_copy.start()
        b1_copy.start()
        w1_copy.start()
        for j in range(len(w2_slabs)):
            w2_copy(j).start()

        def head_matrix(w_ref, rows, h):
            return w_ref[pl.ds(h, rows, stride=H), :]

        x_copy.wait()
        x_f32 = x_v[...].astype(f32)
        x_rows = _batch_rows([x_f32[b:b + 1] for b in range(B)])
        x_ln = _layernorm(x_rows).astype(bf16)

        wq_copy.wait()
        q = [jnp.dot(x_ln, head_matrix(wq_v, M, h),
                     preferred_element_type=f32).astype(bf16)
             for h in range(H)]

        wuk_copy.wait()
        sublane = jax.lax.broadcasted_iota(jnp.int32, (8, C), 0)
        qa = [[None] * (H // 8) for _ in range(B)]
        for h in range(H):
            r = jax.lax.dot_general(q[h], head_matrix(wuk_v, C, h), _NT,
                                    preferred_element_type=f32)
            for b in range(B):
                rb = r[8 * b:8 * b + 8]
                cur = qa[b][h // 8]
                qa[b][h // 8] = rb if cur is None else jnp.where(sublane == h % 8, rb, cur)
        qa = [(jnp.concatenate(qa[b], axis=0) * scale).astype(bf16)
              for b in range(B)]

        ctx_c = []
        for b in range(B):
            def step(i, carry, b=b):
                m, l, acc = carry
                kv_copy(b, i).wait()
                c = ckv_v[b, pl.ds(pl.multiple_of(i * _TK, _TK), _TK), :]
                s = jax.lax.dot_general(qa[b], c, _NT,
                                        preferred_element_type=f32)
                m_new = jnp.maximum(m, jnp.max(s, axis=-1, keepdims=True))
                m_sub = jnp.where(m_new == -jnp.inf, 0.0, m_new)
                alpha = jnp.exp(m - m_sub)
                p = jnp.exp(s - m_sub)
                l = alpha * l + jnp.sum(p, axis=-1, keepdims=True)
                acc = alpha * acc + jnp.dot(p.astype(bf16), c,
                                            preferred_element_type=f32)
                return m_new, l, acc

            init = (jnp.full((H, 1), -jnp.inf, f32),
                    jnp.zeros((H, 1), f32),
                    jnp.zeros((H, C), f32))
            _, l, acc = jax.lax.fori_loop(0, n_kv, step, init)
            ctx_c.append(acc / l)

        wuv_copy.wait()
        ctx = []
        for h in range(H):
            lhs = _batch_rows([ctx_c[b][h:h + 1, :] for b in range(B)]).astype(bf16)
            ctx.append(jnp.dot(lhs, head_matrix(wuv_v, C, h),
                               preferred_element_type=f32).astype(bf16))

        wo_copy.wait()
        attn = jnp.zeros((8 * B, M), f32)
        for h in range(H):
            attn = attn + jnp.dot(ctx[h], wo_v[h], preferred_element_type=f32)
        hidden = x_rows + attn
        row = jax.lax.broadcasted_iota(jnp.int32, (8, M), 0)
        h_res = hidden[0:8]
        for b in range(1, B):
            h_res = jnp.where(row >= b, hidden[8 * b:8 * b + 8], h_res)

        h_ln = _layernorm(h_res).astype(bf16)
        b1_copy.wait()
        w1_copy.wait()
        pre = jnp.dot(h_ln, w1_v[...], preferred_element_type=f32)
        pre = pre + b1_v[...].astype(f32).reshape(1, F)
        softplus = (jnp.log1p(jnp.exp(-jnp.abs(pre)))
                    + jnp.where(pre > 0, pre, jnp.zeros_like(pre)))
        act = (pre * jnp.tanh(softplus)).astype(bf16)

        out = h_res
        for j, (k0, kn) in enumerate(w2_slabs):
            w2_copy(j).wait()
            out = out + jnp.dot(act[:, k0:k0 + kn], w2_v[pl.ds(k0, kn), :],
                                preferred_element_type=f32)
        o_ref[...] = out[0:B, :].astype(o_ref.dtype)

    def kernel(*refs):
        pl.run_scoped(lambda sem: body(*refs, sem), pltpu.SemaphoreType.DMA((n_sem,)))

    hbm = pl.BlockSpec(memory_space=pl.ANY)
    out = pl.pallas_call(
        kernel,
        out_shape=jax.ShapeDtypeStruct((B, M), A_x.dtype),
        in_specs=[hbm] * 9,
        out_specs=pl.BlockSpec(memory_space=pltpu.VMEM),
        scratch_shapes=[
            pltpu.VMEM((B, M), bf16),
            pltpu.VMEM(A_c_kv.shape, bf16),
            pltpu.VMEM((M * H, D), bf16),
            pltpu.VMEM((C * H, D), bf16),
            pltpu.VMEM((C * H, D), bf16),
            pltpu.VMEM(A_w_o.shape, bf16),
            pltpu.VMEM(B_w1.shape, bf16),
            pltpu.VMEM(B_b1.shape, bf16),
            pltpu.VMEM(B_w2.shape, bf16),
        ],
        compiler_params=pltpu.CompilerParams(vmem_limit_bytes=64 * 1024 * 1024),
    )(A_x.reshape(B, M), A_c_kv,
      A_w_q.reshape(M * H, D), A_w_uk.reshape(C * H, D), A_w_uv.reshape(C * H, D),
      A_w_o, B_w1, B_b1, B_w2)
    return out.reshape(B, Sq, M)
```
